```python
import os as _os
_os.environ.setdefault("JAX_PLATFORMS", "cpu")
import jax
import jax.numpy as jnp

def _softmax(x, axis=-1):
    return jax.nn.softmax(x, axis=axis)
def _gelu(x):
    return jax.nn.gelu(x, approximate=True)
def _silu(x):
    return jax.nn.silu(x)
def _sigmoid(x):
    return jax.nn.sigmoid(x)
def _layernorm(x, axis=-1, eps=1e-5):
    m = jnp.mean(x, axis=axis, keepdims=True)
    v = jnp.var(x, axis=axis, keepdims=True)
    return (x - m) / jnp.sqrt(v + eps)
def _scatter_add(tgt, idx, src, axis=0):
    return tgt.at[idx].add(src)
def _segment_sum(src, seg, n):
    return jax.ops.segment_sum(src, seg, n)
class _Rng:
    def __init__(self, key):
        self._k = key
    def _next(self):
        self._k, sub = jax.random.split(self._k)
        return sub
    def normal(self, shape):
        return jax.random.normal(self._next(), shape, dtype=jnp.bfloat16)
    def randint(self, lo, hi, shape):
        return jax.random.randint(self._next(), shape, lo, hi, dtype=jnp.int32)
    def uniform(self, shape, lo=0.0, hi=1.0):
        return jax.random.uniform(self._next(), shape, jnp.bfloat16, lo, hi)
    def permutation(self, n):
        return jax.random.permutation(self._next(), n)


kernel_name = 'sequential_preLN__softmax_full_mha__dense_activation_gelu__prompt'

def setup_inputs():
    _rng = _Rng(jax.random.key(int.from_bytes(__import__("os").urandom(4), "little")))
    _w = (lambda a: (lambda t: t.astype(jnp.bfloat16) if jnp.issubdtype(t.dtype, jnp.floating) else t)(jnp.asarray(a)))
    def _A_setup():
        B, S, D = 1, 2048, 640
        return {
            "x": _w((lambda *s: _rng.normal(s) * 0.05)(B, S, D)),
            "wqkv": _w((lambda *s: _rng.normal(s) * 0.05)(D, 3 * D)),
            "wo": _w((lambda *s: _rng.normal(s) * 0.05)(D, D)),
        }
    _A_in = _A_setup()

    def _B_setup():
        B, S, D, F = 1, 2048, 640, 1536
        return {
            "x": _w((lambda *s: _rng.normal(s) * 0.05)(B, S, D)),
            "w1": _w((lambda *s: _rng.normal(s) * 0.4)(D, F) * (D ** -0.5)),
            "b1": _w((lambda *s: _rng.normal(s) * 0.4)(F) * 0.01),
            "w2": _w((lambda *s: _rng.normal(s) * 0.4)(F, D) * (F ** -0.5)),
            "b2": _w((lambda *s: _rng.normal(s) * 0.05)(D) * 0.01),
        }
    _B_in = _B_setup()

    return {
        "A_x": _A_in["x"],
        "A_wqkv": _A_in["wqkv"],
        "A_wo": _A_in["wo"],
        "B_x": _B_in["x"],
        "B_w1": _B_in["w1"],
        "B_b1": _B_in["b1"],
        "B_w2": _B_in["w2"],
        "B_b2": _B_in["b2"],
    }

def reference(A_x, A_wqkv, A_wo, B_x, B_w1, B_b1, B_w2, B_b2):
    def _A_ref(x, wqkv, wo):
        B, S, D = x.shape
        H = 32; Dh = D // H
        qkv = (lambda x, *d: x.transpose(*d))((x @ wqkv).reshape(B, S, 3, H, Dh), 2, 0, 3, 1, 4)
        q, k, v = qkv[0], qkv[1], qkv[2]
        scale = Dh ** -0.5
        scores = jnp.einsum("bhqd,bhkd->bhqk", q, k) * scale
        p = _softmax(scores, axis=-1)
        o = jnp.einsum("bhqk,bhkd->bhqd", p, v)
        return (lambda x, *d: x.transpose(*d))(o, 0, 2, 1, 3).reshape(B, S, D) @ wo

    def _B_ref(x, w1, b1, w2, b2):
        h = jnp.einsum("bsd,df->bsf", x, w1) + b1
        h = _gelu(h)
        return jnp.einsum("bsf,fd->bsd", h, w2) + b2

    x = A_x
    h = x + _A_ref(_layernorm(x, axis=-1), A_wqkv, A_wo)
    h2 = h + _B_ref(_layernorm(h, axis=-1), B_w1, B_b1, B_w2, B_b2)
    return h2
```

```python
import math

import jax
import jax.numpy as jnp
from jax import lax
import jax.experimental.pallas as pl
import jax.experimental.pallas.tpu as pltpu

S, D, H, DH, F = 2048, 640, 32, 20, 1536
NSLAB = D // 128
EPS = 1e-5
QSCALE = (DH ** -0.5) * math.log2(math.e)
NN = (((1,), (0,)), ((), ()))
NT = (((1,), (1,)), ((), ()))
TN = (((0,), (0,)), ((), ()))
f32 = jnp.float32
bf16 = jnp.bfloat16
u32 = jnp.uint32

L_LO = 2.0 ** -80
L_HI = 2.0 ** 60
V_HI = 2.0 ** 60

TQ = 512
TK = 128
XC = 16
MC = TK - XC
NG = XC // 8
DP = DH // 2
RB = 256
NH = 2
FC = 384
FB = 256
NQ = S // TQ
NC = S // TK
NR = S // RB
HR = TQ // NH
NJ = TQ // 128
NF = F // FC
NLAST = 2
NPRE = 4
G0A, G0, G1, G2, G3 = 1, 3, 3, 3, 2
assert G0 + (NR - 2) * G1 + G2 + NQ * G3 == NC * NG


def _ln(x):
    m = jnp.mean(x, axis=-1, keepdims=True)
    xc = x - m
    v = jnp.mean(xc * xc, axis=-1, keepdims=True)
    return xc * lax.rsqrt(v + EPS)


def _gelu(x):
    c = math.sqrt(2.0 / math.pi)
    return 0.5 * x * (1.0 + jnp.tanh(c * (x + 0.044715 * (x * x * x))))


def _ds(start, n, align):
    if isinstance(start, int):
        return pl.ds(start, n)
    return pl.ds(pl.multiple_of(start, align), n)


def _regroup(a, gsz):
    per = TK // 16
    parts = []
    for g in range(a.shape[0] // gsz):
        cb, gi = divmod(g, per)
        src = cb * per + (MC // 16 - 1 - gi if gi < MC // 16 else gi)
        parts.append(a[src * gsz:(src + 1) * gsz, :])
    return jnp.concatenate(parts, axis=0)


def _kernel(x_hbm, wqkv_hbm, wo_hbm, w1_hbm, b1_ref, w2_hbm, b2_ref, o_hbm,
            x_v, wqkv_v, wo_v, w1_v, w2_v, sems, osems,
            kc_scr, k_scr, vt_scr, wt_scr, p_scr, raw_scr, qta_scr, qtb_scr, kb_scr,
            flag_ref, z_ref, acc_scr, s_scr, vok_scr):
    i = pl.program_id(0)
    qts = (qta_scr, qtb_scr)

    def x_copy(r):
        rows = _ds(r * RB, RB, RB)
        return pltpu.make_async_copy(x_hbm.at[rows], x_v.at[rows], sems.at[6 + r])

    def w_copy(j):
        cols = pl.ds(j * D, D)
        return pltpu.make_async_copy(wqkv_hbm.at[:, cols], wqkv_v.at[:, cols], sems.at[j])

    wo_copy = pltpu.make_async_copy(wo_hbm, wo_v, sems.at[3])
    w1_copy = pltpu.make_async_copy(w1_hbm, w1_v, sems.at[4])
    w2_copy = pltpu.make_async_copy(w2_hbm, w2_v, sems.at[5])

    def rot_k(h, r0, n):
        c0 = h * DH
        lo = c0 % 128
        sl = c0 // 128 + jnp.where(lo > 128 - DH, NSLAB, 0)
        rows2 = _ds(r0 // 2, n // 2, 8)
        kk = pltpu.roll(k_scr[sl, rows2, :], (128 - lo) & 127, 1)
        kc_scr[rows2, :] = _regroup(kk, 8)

    def qk_dot(qm, rows2):
        lhs = pltpu.bitcast(kc_scr[rows2, :], bf16)[:, 0:DH]
        return _regroup(lax.dot_general(lhs, qm, NN, preferred_element_type=f32), 16)

    def vpu_piece(h, c, qs):
        groups = []
        for g in range(NG):
            def step(dp, accs, g=g):
                w = kb_scr[h * DP + dp, _ds(c * XC + g * 8, 8, 8), :]
                kbs = (pltpu.bitcast(w << 16, f32), pltpu.bitcast(w & u32(0xFFFF0000), f32))
                accs = list(accs)
                for e in range(2):
                    for j in range(NJ):
                        c0 = qs * TQ + j * 128
                        qrow = qts[g][h, pl.ds(2 * dp + e, 1), c0:c0 + 128]
                        t = kbs[e] * jnp.broadcast_to(qrow, (8, 128))
                        accs[j] = t if accs[j] is None else accs[j] + t
                return tuple(accs)

            accs = step(0, (None,) * NJ)
            accs = lax.fori_loop(1, DP, step, accs, unroll=True)
            groups.append(jnp.concatenate(accs, axis=1))
        return jnp.concatenate(groups, axis=0)

    def pv_dot(h, c, qs, acc):
        keys = _ds(c * TK, TK, TK)
        pv = lax.dot_general(vt_scr[h, :, keys], p_scr[qs, keys, :], NN, preferred_element_type=f32)
        return pv if acc is None else acc + pv

    def check_tile(qs):
        sub = lax.broadcasted_iota(jnp.int32, (8, TQ), 0)
        good = vok_scr[...]
        for p in range(H // 2):
            lboth = jnp.where(sub < 4, raw_scr[qs, 2 * p + 1, 0:8, :], raw_scr[qs, 2 * p, 16:24, :])
            good = jnp.where(jnp.logical_and(lboth >= L_LO, lboth <= L_HI), good, 0.0)
        flag_ref[0] = jnp.min(good)

    def attn_out_t(qs, cols):
        n = cols.stop - cols.start
        sub = lax.broadcasted_iota(jnp.int32, (8, n), 0)
        blks = []
        for p in range(H // 2):
            ae = raw_scr[qs, 2 * p, :, cols]
            ao = raw_scr[qs, 2 * p + 1, :, cols]
            lboth = jnp.where(sub < 4, ao[0:8, :], ae[16:24, :])
            r0 = pl.reciprocal(lboth, approx=True)
            inv = r0 * (2.0 - lboth * r0)
            inv = inv * (2.0 - lboth * inv)
            oe = ae * inv[7:8, :]
            oo = ao * inv[0:1, :]
            blks += [oe[0:16, :], jnp.where(sub < 4, oe[16:24, :], oo[0:8, :]), oo[8:24, :]]
        return jnp.concatenate(blks, axis=0)

    def ln_block(r):
        return _ln(x_v[_ds(r * RB, RB, RB), :].astype(f32)).astype(bf16)

    def proj_k(r, xn):
        lane = lax.broadcasted_iota(jnp.int32, (RB, 128), 1)
        k = jnp.dot(xn, wqkv_v[:, D:2 * D], preferred_element_type=f32)
        ks = [k[:, 128 * s:128 * (s + 1)] for s in range(NSLAB)]
        rows2 = _ds(r * (RB // 2), RB // 2, RB // 2)
        for s in range(NSLAB):
            k_scr[s, rows2, :] = pltpu.bitcast(ks[s].astype(bf16), u32)
        for s in range(NSLAB - 1):
            merged = jnp.where(lane < 64, ks[s + 1], ks[s])
            k_scr[NSLAB + s, rows2, :] = pltpu.bitcast(merged.astype(bf16), u32)

    def gen_kb(v0, n):
        ws = []
        for t in range(n):
            v = v0 + t
            c = v // NG
            g = v % NG
            krows = _ds((c * TK + MC) // 2, 8, 8)
            row = []
            for s in range(NSLAB):
                kf = pltpu.bitcast(k_scr[s, krows, :], bf16).astype(f32)
                kf = jnp.where(g == 0, kf[0:8, :], kf[8:16, :])
                bits = pltpu.bitcast(kf, u32)
                row.append((bits >> 16) | pltpu.roll(bits, 127, 1))
            ws.append(row)
        xrows = _ds(v0 * 8, 8 * n, 8)
        wcat = [jnp.concatenate([ws[t][s] for t in range(n)], axis=0) for s in range(NSLAB)]
        for l in range(0, 128, 2):
            for s in range(NSLAB):
                kb_scr[(128 * s + l) // 2, xrows, :] = jnp.broadcast_to(wcat[s][:, l:l + 1], (8 * n, 128))

    def proj_qv(r, xn, first=False):
        rows = _ds(r * RB, RB, RB)
        sub_r = lax.broadcasted_iota(jnp.int32, (8, RB), 0)
        qvt = lax.dot_general(wt_scr[...], xn, NT, preferred_element_type=f32)
        qt32 = qvt[0:D, :] * QSCALE
        for h in range(H):
            qh = qt32[DH * h:DH * (h + 1), :]
            qta_scr[h, :, rows] = qh
            qtb_scr[h, :, rows] = qh
        vm = jnp.max(jnp.abs(qvt[D:2 * D, :]).reshape(D // 8, 8, RB), axis=0)
        vm = jnp.concatenate([vm] * (TQ // RB), axis=1)
        vprev = 1.0 if first else vok_scr[...]
        vok_scr[...] = jnp.where(vm <= V_HI, vprev, 0.0)
        for h in range(H):
            if h % 2 == 0:
                off = D + DH * h
                blk = [qvt[off:off + 16, :], jnp.where(sub_r < 4, qvt[off + 16:off + 24, :], 1.0)]
            else:
                off = D + DH * h - 4
                blk = [jnp.where(sub_r >= 4, qvt[off:off + 8, :], 1.0), qvt[off + 8:off + 24, :]]
            vt_scr[h, :, rows] = jnp.concatenate(blk, axis=0)

    @pl.when(i == 0)
    def _attention():
        x_copy(0).start()
        w_copy(1).start()
        x_copy(1).start()
        x_copy(0).wait()
        w_copy(0).start()
        w_copy(2).start()
        xn0 = ln_block(0)
        w_copy(1).wait()
        x_copy(1).wait()
        x_copy(2).start()
        proj_k(0, xn0)
        xn1 = ln_block(1)
        gen_kb(0, G0A)
        proj_k(1, xn1)
        w_copy(0).wait()
        w_copy(2).wait()
        for r in range(3, NR):
            x_copy(r).start()
        wo_copy.start()
        w1_copy.start()
        w2_copy.start()
        gen_kb(G0A, G0 - G0A)
        wt_scr[0:D, :] = wqkv_v[:, 0:D].astype(f32).T.astype(bf16)
        wt_scr[D:2 * D, :] = wqkv_v[:, 2 * D:3 * D].astype(f32).T.astype(bf16)
        proj_qv(0, xn0, first=True)

        def rb_body(r, xn):
            x_copy(r + 1).wait()
            gen_kb(G0 + (r - 1) * G1, G1)
            xn_next = ln_block(r + 1)
            proj_qv(r, xn)
            proj_k(r + 1, xn_next)
            return xn_next

        xn_last = lax.fori_loop(1, NR - 1, rb_body, xn1)
        rot_k(1, 0, S)
        gen_kb(G0 + (NR - 2) * G1, G2)
        proj_qv(NR - 1, xn_last)

        z_ref[0] = 0
        z_ref[1] = 0

        def first_body(qs, carry):
            gen_kb(G0 + (NR - 2) * G1 + G2 + qs * G3, G3)
            qm = qta_scr[0, :, _ds(qs * TQ, TQ, TQ)]
            for c in range(NC):
                lhs = pltpu.bitcast(k_scr[0, c * TK // 2:(c + 1) * TK // 2, :], bf16)[:, 0:DH]
                s = lax.dot_general(lhs, qm, NN, preferred_element_type=f32)
                p_scr[qs, c * TK:(c + 1) * TK, :] = jnp.exp2(s)
            return carry

        lax.fori_loop(0, NQ, first_body, 0)

        def head_body(h, carry):
            h2 = jnp.minimum(h + 2, H - 1)
            z1 = z_ref[0]
            z2 = z_ref[1]
            qms = [qta_scr[h + 1, :, qs * TQ:(qs + 1) * TQ] for qs in range(NQ)]

            def issue(qs, c, n):
                sm = qk_dot(qms[qs], _ds(c * (TK // 2), n // 2, 8))
                if qs == NQ - 1:
                    rot_k(h2, c * TK, n)
                return sm

            def retire(qs, c, sm, first=False, last=False):
                acc = pv_dot(h, c, qs, None if first else acc_scr[z1])
                if last:
                    raw_scr[qs, h] = acc
                else:
                    acc_scr[z2] = acc
                if sm.shape[0] == MC:
                    p_scr[qs, _ds(c * TK + MC, XC, XC), :] = jnp.exp2(vpu_piece(h + 1, c, qs))
                p_scr[qs, _ds(c * TK, sm.shape[0], TK), :] = jnp.exp2(sm)

            sm = issue(0, 0, MC)
            for qs in range(NQ):
                lastq = qs == NQ - 1
                nxt = issue(qs, 1, MC)
                retire(qs, 0, sm, first=True)

                def mid(c, cur, qs=qs):
                    nx = issue(qs, c + 1, MC)
                    retire(qs, c, cur)
                    return nx

                hi = NC - 1 - (NLAST if lastq else 0)
                sm = lax.fori_loop(1, hi, mid, nxt, unroll=True)
                for c in range(hi, NC):
                    if c + 1 < NC:
                        nxt = issue(qs, c + 1, TK)
                    elif not lastq:
                        nxt = issue(qs + 1, 0, MC)
                    retire(qs, c, sm, last=(c == NC - 1))
                    sm = nxt
            return carry

        lax.fori_loop(0, H - 1, head_body, 0)

        acc = None
        for c in range(NC):
            acc = pv_dot(H - 1, c, 0, acc)
        raw_scr[0, H - 1] = acc
        check_tile(0)

        wo_copy.wait()
        w1_copy.wait()
        w2_copy.wait()

    @pl.when(flag_ref[0] < 0.5)
    def _fallback():
        def fb_head(h, carry):
            rot_k(h, 0, S)
            qm = qta_scr[h, :, _ds(i * TQ, TQ, TQ)]

            def pass1(c, m8):
                s = qk_dot(qm, _ds(c * (FB // 2), FB // 2, FB // 2))
                s_scr[_ds(c * FB, FB, FB), :] = s
                return jnp.maximum(m8, jnp.max(s.reshape(FB // 8, 8, TQ), axis=0))

            m8 = lax.fori_loop(0, S // FB, pass1, jnp.full((8, TQ), -jnp.inf, f32))
            m = jnp.max(m8, axis=0, keepdims=True)

            def pass2(c, acc):
                rows = _ds(c * FB, FB, FB)
                p = jnp.exp2(s_scr[rows, :] - m)
                return acc + lax.dot_general(vt_scr[h, :, rows], p, NN, preferred_element_type=f32)

            raw_scr[i, h] = lax.fori_loop(0, S // FB, pass2, jnp.zeros((24, TQ), f32))
            return carry

        lax.fori_loop(0, H, fb_head, 0)

    b1 = b1_ref[...].astype(f32).reshape(1, F)
    b2 = b2_ref[...].astype(f32).reshape(1, D)
    qn = jnp.minimum(i + 1, NQ - 1)
    st = dict(u=0, acc=None, dots=0)

    def pv_until(tgt):
        while st["u"] < tgt:
            st["acc"] = pv_dot(H - 1, st["u"], qn, st["acc"])
            st["u"] += 1
            if st["u"] == NC:
                raw_scr[qn, H - 1] = st["acc"]
                check_tile(qn)

    def after_dot():
        st["dots"] += 1
        pv_until(min(NC, NPRE + -(-(NC - NPRE) * st["dots"] // (2 * NH * NF - 4))))

    pv_until(NPRE)
    hres = []
    for a in range(NH):
        ot = attn_out_t(i, slice(a * HR, (a + 1) * HR)).astype(bf16)
        attn = lax.dot_general(ot, wo_v[...], TN, preferred_element_type=f32)
        hres.append(x_v[_ds(i * TQ + a * HR, HR, HR), :].astype(f32) + attn)
    gs = []
    for a in range(NH):
        hn = _ln(hres[a]).astype(bf16)
        row = []
        for n in range(NF):
            cols = slice(n * FC, (n + 1) * FC)
            act = jnp.dot(hn, w1_v[:, cols], preferred_element_type=f32) + b1[:, cols]
            row.append(_gelu(act).astype(bf16))
            after_dot()
        gs.append(row)
    for a in range(NH):
        y = hres[a] + b2
        for n in range(NF):
            y = y + jnp.dot(gs[a][n], w2_v[n * FC:(n + 1) * FC, :], preferred_element_type=f32)
            after_dot()
        orows = _ds(i * TQ + a * HR, HR, HR)
        x_v[orows, :] = y.astype(bf16)
        pltpu.make_async_copy(x_v.at[orows], o_hbm.at[orows], osems.at[i * NH + a]).start()

    @pl.when(i == NQ - 1)
    def _drain():
        for t in range(NQ * NH):
            rr = pl.ds(t * HR, HR)
            pltpu.make_async_copy(x_v.at[rr], o_hbm.at[rr], osems.at[t]).wait()


@jax.jit
def pallas_sequential_preLN__softmax_full_mha__dense_activation_gelu__prompt_kernel(
    A_x: jax.Array,
    A_wqkv: jax.Array,
    A_wo: jax.Array,
    B_x: jax.Array,
    B_w1: jax.Array,
    B_b1: jax.Array,
    B_w2: jax.Array,
    B_b2: jax.Array,
):
    del B_x
    hbm = pl.BlockSpec(memory_space=pl.ANY)
    out = pl.pallas_call(
        _kernel,
        grid=(NQ,),
        in_specs=[hbm, hbm, hbm, hbm,
                  pl.BlockSpec((F,), lambda i: (0,)), hbm, pl.BlockSpec((D,), lambda i: (0,))],
        out_specs=hbm,
        out_shape=jax.ShapeDtypeStruct((S, D), bf16),
        scratch_shapes=[
            pltpu.VMEM((S, D), bf16),
            pltpu.VMEM((D, 3 * D), bf16),
            pltpu.VMEM((D, D), bf16),
            pltpu.VMEM((D, F), bf16),
            pltpu.VMEM((F, D), bf16),
            pltpu.SemaphoreType.DMA((6 + NR,)),
            pltpu.SemaphoreType.DMA((NQ * NH,)),
            pltpu.VMEM((S // 2, 128), u32),
            pltpu.VMEM((2 * NSLAB - 1, S // 2, 128), u32),
            pltpu.VMEM((H, 24, S), f32),
            pltpu.VMEM((2 * D, D), bf16),
            pltpu.VMEM((NQ, S, TQ), f32),
            pltpu.VMEM((NQ, H, 24, TQ), f32),
            pltpu.VMEM((H, DH, S), f32),
            pltpu.VMEM((H, DH, S), f32),
            pltpu.VMEM((D // 2, NC * XC, 128), u32),
            pltpu.SMEM((1,), f32),
            pltpu.SMEM((2,), jnp.int32),
            pltpu.VMEM((2, 24, TQ), f32),
            pltpu.VMEM((S, TQ), f32),
            pltpu.VMEM((8, TQ), f32),
        ],
        compiler_params=pltpu.CompilerParams(
            dimension_semantics=("arbitrary",),
            vmem_limit_bytes=120 * 1024 * 1024,
        ),
    )(A_x.reshape(S, D), A_wqkv, A_wo, B_w1, B_b1, B_w2, B_b2)
    return out.reshape(1, S, D)
```

```python
import math

import jax
import jax.numpy as jnp
from jax import lax
import jax.experimental.pallas as pl
import jax.experimental.pallas.tpu as pltpu

S, D, H, DH, F = 2048, 640, 32, 20, 1536
NSLAB = D // 128
EPS = 1e-5
QSCALE = (DH ** -0.5) * math.log2(math.e)
NN = (((1,), (0,)), ((), ()))
NT = (((1,), (1,)), ((), ()))
TN = (((0,), (0,)), ((), ()))
f32 = jnp.float32
bf16 = jnp.bfloat16
u32 = jnp.uint32

L_LO = 2.0 ** -80
L_HI = 2.0 ** 60
V_HI = 2.0 ** 60

TQ = 512
TK = 128
XC = 16
MC = TK - XC
NG = XC // 8
DP = DH // 2
RB = 256
NH = 2
FC = 384
FB = 256
NQ = S // TQ
NC = S // TK
NR = S // RB
HR = TQ // NH
NJ = TQ // 128
NF = F // FC
NLAST = 2
NPRE = 4
G0A, G0, G1, G2, G3 = 1, 3, 3, 3, 2
assert G0 + (NR - 2) * G1 + G2 + NQ * G3 == NC * NG


def _ln(x):
    m = jnp.mean(x, axis=-1, keepdims=True)
    xc = x - m
    v = jnp.mean(xc * xc, axis=-1, keepdims=True)
    return xc * lax.rsqrt(v + EPS)


def _gelu(x):
    c = math.sqrt(2.0 / math.pi)
    return 0.5 * x * (1.0 + jnp.tanh(c * (x + 0.044715 * (x * x * x))))


def _ds(start, n, align):
    if isinstance(start, int):
        return pl.ds(start, n)
    return pl.ds(pl.multiple_of(start, align), n)


def _regroup(a, gsz):
    per = TK // 16
    parts = []
    for g in range(a.shape[0] // gsz):
        cb, gi = divmod(g, per)
        src = cb * per + (MC // 16 - 1 - gi if gi < MC // 16 else gi)
        parts.append(a[src * gsz:(src + 1) * gsz, :])
    return jnp.concatenate(parts, axis=0)


def _kernel(x_hbm, wqkv_hbm, wo_hbm, w1_hbm, b1_ref, w2_hbm, b2_ref, o_hbm,
            x_v, wq_v, wk_v, wv_v, wo_v, w1_v, w2_v, sems, osems,
            kc_scr, k_scr, vt_scr, wt_scr, p_scr, raw_scr, qta_scr, qtb_scr, kb_scr,
            flag_ref, z_ref, acc_scr, s_scr, vok_scr):
    i = pl.program_id(0)
    qts = (qta_scr, qtb_scr)

    def x_copy(r):
        rows = _ds(r * RB, RB, RB)
        return pltpu.make_async_copy(x_hbm.at[rows], x_v.at[rows], sems.at[6 + r])

    def w_copy(j):
        dst = (wq_v, wk_v, wv_v)[j]
        return pltpu.make_async_copy(wqkv_hbm.at[:, pl.ds(j * D, D)], dst, sems.at[j])

    wo_copy = pltpu.make_async_copy(wo_hbm, wo_v, sems.at[3])
    w1_copy = pltpu.make_async_copy(w1_hbm, w1_v, sems.at[4])
    w2_copy = pltpu.make_async_copy(w2_hbm, w2_v, sems.at[5])

    def rot_k(h, r0, n):
        c0 = h * DH
        lo = c0 % 128
        sl = c0 // 128 + jnp.where(lo > 128 - DH, NSLAB, 0)
        rows2 = _ds(r0 // 2, n // 2, 8)
        kk = pltpu.roll(k_scr[sl, rows2, :], (128 - lo) & 127, 1)
        kc_scr[rows2, :] = _regroup(kk, 8)

    def qk_dot(qm, rows2):
        lhs = pltpu.bitcast(kc_scr[rows2, :], bf16)[:, 0:DH]
        return _regroup(lax.dot_general(lhs, qm, NN, preferred_element_type=f32), 16)

    def vpu_piece(h, c, qs):
        groups = []
        for g in range(NG):
            def step(dp, accs, g=g):
                w = kb_scr[h * DP + dp, _ds(c * XC + g * 8, 8, 8), :]
                kbs = (pltpu.bitcast(w << 16, f32), pltpu.bitcast(w & u32(0xFFFF0000), f32))
                accs = list(accs)
                for e in range(2):
                    for j in range(NJ):
                        c0 = qs * TQ + j * 128
                        qrow = qts[g][h, pl.ds(2 * dp + e, 1), c0:c0 + 128]
                        t = kbs[e] * jnp.broadcast_to(qrow, (8, 128))
                        accs[j] = t if accs[j] is None else accs[j] + t
                return tuple(accs)

            accs = step(0, (None,) * NJ)
            accs = lax.fori_loop(1, DP, step, accs, unroll=True)
            groups.append(jnp.concatenate(accs, axis=1))
        return jnp.concatenate(groups, axis=0)

    def pv_dot(h, c, qs, acc):
        keys = _ds(c * TK, TK, TK)
        pv = lax.dot_general(vt_scr[h, :, keys], p_scr[qs, keys, :], NN, preferred_element_type=f32)
        return pv if acc is None else acc + pv

    def check_tile(qs):
        sub = lax.broadcasted_iota(jnp.int32, (8, TQ), 0)
        good = vok_scr[...]
        for p in range(H // 2):
            lboth = jnp.where(sub < 4, raw_scr[qs, 2 * p + 1, 0:8, :], raw_scr[qs, 2 * p, 16:24, :])
            good = jnp.where(jnp.logical_and(lboth >= L_LO, lboth <= L_HI), good, 0.0)
        flag_ref[0] = jnp.min(good)

    def attn_out_t(qs, cols):
        n = cols.stop - cols.start
        sub = lax.broadcasted_iota(jnp.int32, (8, n), 0)
        blks = []
        for p in range(H // 2):
            ae = raw_scr[qs, 2 * p, :, cols]
            ao = raw_scr[qs, 2 * p + 1, :, cols]
            lboth = jnp.where(sub < 4, ao[0:8, :], ae[16:24, :])
            r0 = pl.reciprocal(lboth, approx=True)
            inv = r0 * (2.0 - lboth * r0)
            inv = inv * (2.0 - lboth * inv)
            oe = ae * inv[7:8, :]
            oo = ao * inv[0:1, :]
            blks += [oe[0:16, :], jnp.where(sub < 4, oe[16:24, :], oo[0:8, :]), oo[8:24, :]]
        return jnp.concatenate(blks, axis=0)

    def ln_block(r):
        return _ln(x_v[_ds(r * RB, RB, RB), :].astype(f32)).astype(bf16)

    def proj_k(r, xn):
        lane = lax.broadcasted_iota(jnp.int32, (RB, 128), 1)
        k = jnp.dot(xn, wk_v[...], preferred_element_type=f32)
        ks = [k[:, 128 * s:128 * (s + 1)] for s in range(NSLAB)]
        rows2 = _ds(r * (RB // 2), RB // 2, RB // 2)
        for s in range(NSLAB):
            k_scr[s, rows2, :] = pltpu.bitcast(ks[s].astype(bf16), u32)
        for s in range(NSLAB - 1):
            merged = jnp.where(lane < 64, ks[s + 1], ks[s])
            k_scr[NSLAB + s, rows2, :] = pltpu.bitcast(merged.astype(bf16), u32)

    def gen_kb(v0, n):
        ws = []
        for t in range(n):
            v = v0 + t
            c = v // NG
            g = v % NG
            krows = _ds((c * TK + MC) // 2, 8, 8)
            row = []
            for s in range(NSLAB):
                kf = pltpu.bitcast(k_scr[s, krows, :], bf16).astype(f32)
                kf = jnp.where(g == 0, kf[0:8, :], kf[8:16, :])
                bits = pltpu.bitcast(kf, u32)
                row.append((bits >> 16) | pltpu.roll(bits, 127, 1))
            ws.append(row)
        xrows = _ds(v0 * 8, 8 * n, 8)
        wcat = [jnp.concatenate([ws[t][s] for t in range(n)], axis=0) for s in range(NSLAB)]
        for l in range(0, 128, 2):
            for s in range(NSLAB):
                kb_scr[(128 * s + l) // 2, xrows, :] = jnp.broadcast_to(wcat[s][:, l:l + 1], (8 * n, 128))

    def proj_qv(r, xn, first=False):
        rows = _ds(r * RB, RB, RB)
        sub_r = lax.broadcasted_iota(jnp.int32, (8, RB), 0)
        qvt = lax.dot_general(wt_scr[...], xn, NT, preferred_element_type=f32)
        qt32 = qvt[0:D, :] * QSCALE
        for h in range(H):
            qh = qt32[DH * h:DH * (h + 1), :]
            qta_scr[h, :, rows] = qh
            qtb_scr[h, :, rows] = qh
        vm = jnp.max(jnp.abs(qvt[D:2 * D, :]).reshape(D // 8, 8, RB), axis=0)
        vm = jnp.concatenate([vm] * (TQ // RB), axis=1)
        vprev = 1.0 if first else vok_scr[...]
        vok_scr[...] = jnp.where(vm <= V_HI, vprev, 0.0)
        for h in range(H):
            if h % 2 == 0:
                off = D + DH * h
                blk = [qvt[off:off + 16, :], jnp.where(sub_r < 4, qvt[off + 16:off + 24, :], 1.0)]
            else:
                off = D + DH * h - 4
                blk = [jnp.where(sub_r >= 4, qvt[off:off + 8, :], 1.0), qvt[off + 8:off + 24, :]]
            vt_scr[h, :, rows] = jnp.concatenate(blk, axis=0)

    @pl.when(i == 0)
    def _attention():
        x_copy(0).start()
        w_copy(1).start()
        x_copy(1).start()
        x_copy(0).wait()
        w_copy(0).start()
        w_copy(2).start()
        xn0 = ln_block(0)
        w_copy(1).wait()
        x_copy(1).wait()
        x_copy(2).start()
        proj_k(0, xn0)
        xn1 = ln_block(1)
        gen_kb(0, G0A)
        proj_k(1, xn1)
        w_copy(0).wait()
        w_copy(2).wait()
        for r in range(3, NR):
            x_copy(r).start()
        wo_copy.start()
        w1_copy.start()
        w2_copy.start()
        gen_kb(G0A, G0 - G0A)
        wt_scr[0:D, :] = wq_v[...].astype(f32).T.astype(bf16)
        wt_scr[D:2 * D, :] = wv_v[...].astype(f32).T.astype(bf16)
        proj_qv(0, xn0, first=True)

        def rb_body(r, xn):
            x_copy(r + 1).wait()
            gen_kb(G0 + (r - 1) * G1, G1)
            xn_next = ln_block(r + 1)
            proj_qv(r, xn)
            proj_k(r + 1, xn_next)
            return xn_next

        xn_last = lax.fori_loop(1, NR - 1, rb_body, xn1)
        rot_k(1, 0, S)
        gen_kb(G0 + (NR - 2) * G1, G2)
        proj_qv(NR - 1, xn_last)

        z_ref[0] = 0
        z_ref[1] = 0

        def first_body(qs, carry):
            gen_kb(G0 + (NR - 2) * G1 + G2 + qs * G3, G3)
            qm = qta_scr[0, :, _ds(qs * TQ, TQ, TQ)]
            for c in range(NC):
                lhs = pltpu.bitcast(k_scr[0, c * TK // 2:(c + 1) * TK // 2, :], bf16)[:, 0:DH]
                s = lax.dot_general(lhs, qm, NN, preferred_element_type=f32)
                p_scr[qs, c * TK:(c + 1) * TK, :] = jnp.exp2(s)
            return carry

        lax.fori_loop(0, NQ, first_body, 0)

        def head_body(h, carry):
            h2 = jnp.minimum(h + 2, H - 1)
            z1 = z_ref[0]
            z2 = z_ref[1]
            qms = [qta_scr[h + 1, :, qs * TQ:(qs + 1) * TQ] for qs in range(NQ)]

            def issue(qs, c, n):
                sm = qk_dot(qms[qs], _ds(c * (TK // 2), n // 2, 8))
                if qs == NQ - 1:
                    rot_k(h2, c * TK, n)
                return sm

            def retire(qs, c, sm, first=False, last=False):
                acc = pv_dot(h, c, qs, None if first else acc_scr[z1])
                if last:
                    raw_scr[qs, h] = acc
                else:
                    acc_scr[z2] = acc
                if sm.shape[0] == MC:
                    p_scr[qs, _ds(c * TK + MC, XC, XC), :] = jnp.exp2(vpu_piece(h + 1, c, qs))
                p_scr[qs, _ds(c * TK, sm.shape[0], TK), :] = jnp.exp2(sm)

            sm = issue(0, 0, MC)
            for qs in range(NQ):
                lastq = qs == NQ - 1
                nxt = issue(qs, 1, MC)
                retire(qs, 0, sm, first=True)

                def mid(c, cur, qs=qs):
                    nx = issue(qs, c + 1, MC)
                    retire(qs, c, cur)
                    return nx

                hi = NC - 1 - (NLAST if lastq else 0)
                sm = lax.fori_loop(1, hi, mid, nxt, unroll=True)
                for c in range(hi, NC):
                    if c + 1 < NC:
                        nxt = issue(qs, c + 1, TK)
                    elif not lastq:
                        nxt = issue(qs + 1, 0, MC)
                    retire(qs, c, sm, last=(c == NC - 1))
                    sm = nxt
            return carry

        lax.fori_loop(0, H - 1, head_body, 0)

        acc = None
        for c in range(NC):
            acc = pv_dot(H - 1, c, 0, acc)
        raw_scr[0, H - 1] = acc
        check_tile(0)

        wo_copy.wait()
        w1_copy.wait()
        w2_copy.wait()

    @pl.when(flag_ref[0] < 0.5)
    def _fallback():
        def fb_head(h, carry):
            rot_k(h, 0, S)
            qm = qta_scr[h, :, _ds(i * TQ, TQ, TQ)]

            def pass1(c, m8):
                s = qk_dot(qm, _ds(c * (FB // 2), FB // 2, FB // 2))
                s_scr[_ds(c * FB, FB, FB), :] = s
                return jnp.maximum(m8, jnp.max(s.reshape(FB // 8, 8, TQ), axis=0))

            m8 = lax.fori_loop(0, S // FB, pass1, jnp.full((8, TQ), -jnp.inf, f32))
            m = jnp.max(m8, axis=0, keepdims=True)

            def pass2(c, acc):
                rows = _ds(c * FB, FB, FB)
                p = jnp.exp2(s_scr[rows, :] - m)
                return acc + lax.dot_general(vt_scr[h, :, rows], p, NN, preferred_element_type=f32)

            raw_scr[i, h] = lax.fori_loop(0, S // FB, pass2, jnp.zeros((24, TQ), f32))
            return carry

        lax.fori_loop(0, H, fb_head, 0)

    b1 = b1_ref[...].astype(f32).reshape(1, F)
    b2 = b2_ref[...].astype(f32).reshape(1, D)
    qn = jnp.minimum(i + 1, NQ - 1)
    st = dict(u=0, acc=None, dots=0)

    def pv_until(tgt):
        while st["u"] < tgt:
            st["acc"] = pv_dot(H - 1, st["u"], qn, st["acc"])
            st["u"] += 1
            if st["u"] == NC:
                raw_scr[qn, H - 1] = st["acc"]
                check_tile(qn)

    def after_dot():
        st["dots"] += 1
        pv_until(min(NC, NPRE + -(-(NC - NPRE) * st["dots"] // (2 * NH * NF - 4))))

    pv_until(NPRE)
    hres = []
    for a in range(NH):
        ot = attn_out_t(i, slice(a * HR, (a + 1) * HR)).astype(bf16)
        attn = lax.dot_general(ot, wo_v[...], TN, preferred_element_type=f32)
        hres.append(x_v[_ds(i * TQ + a * HR, HR, HR), :].astype(f32) + attn)
    gs = []
    for a in range(NH):
        hn = _ln(hres[a]).astype(bf16)
        row = []
        for n in range(NF):
            cols = slice(n * FC, (n + 1) * FC)
            act = jnp.dot(hn, w1_v[:, cols], preferred_element_type=f32) + b1[:, cols]
            row.append(_gelu(act).astype(bf16))
            after_dot()
        gs.append(row)
    for a in range(NH):
        y = hres[a] + b2
        for n in range(NF):
            y = y + jnp.dot(gs[a][n], w2_v[n * FC:(n + 1) * FC, :], preferred_element_type=f32)
            after_dot()
        orows = _ds(i * TQ + a * HR, HR, HR)
        x_v[orows, :] = y.astype(bf16)
        pltpu.make_async_copy(x_v.at[orows], o_hbm.at[orows], osems.at[i * NH + a]).start()

    @pl.when(i == NQ - 1)
    def _drain():
        for t in range(NQ * NH):
            rr = pl.ds(t * HR, HR)
            pltpu.make_async_copy(x_v.at[rr], o_hbm.at[rr], osems.at[t]).wait()


@jax.jit
def pallas_sequential_preLN__softmax_full_mha__dense_activation_gelu__prompt_kernel(
    A_x: jax.Array,
    A_wqkv: jax.Array,
    A_wo: jax.Array,
    B_x: jax.Array,
    B_w1: jax.Array,
    B_b1: jax.Array,
    B_w2: jax.Array,
    B_b2: jax.Array,
):
    del B_x
    hbm = pl.BlockSpec(memory_space=pl.ANY)
    out = pl.pallas_call(
        _kernel,
        grid=(NQ,),
        in_specs=[hbm, hbm, hbm, hbm,
                  pl.BlockSpec((F,), lambda i: (0,)), hbm, pl.BlockSpec((D,), lambda i: (0,))],
        out_specs=hbm,
        out_shape=jax.ShapeDtypeStruct((S, D), bf16),
        scratch_shapes=[
            pltpu.VMEM((S, D), bf16),
            pltpu.VMEM((D, D), bf16),
            pltpu.VMEM((D, D), bf16),
            pltpu.VMEM((D, D), bf16),
            pltpu.VMEM((D, D), bf16),
            pltpu.VMEM((D, F), bf16),
            pltpu.VMEM((F, D), bf16),
            pltpu.SemaphoreType.DMA((6 + NR,)),
            pltpu.SemaphoreType.DMA((NQ * NH,)),
            pltpu.VMEM((S // 2, 128), u32),
            pltpu.VMEM((2 * NSLAB - 1, S // 2, 128), u32),
            pltpu.VMEM((H, 24, S), f32),
            pltpu.VMEM((2 * D, D), bf16),
            pltpu.VMEM((NQ, S, TQ), f32),
            pltpu.VMEM((NQ, H, 24, TQ), f32),
            pltpu.VMEM((H, DH, S), f32),
            pltpu.VMEM((H, DH, S), f32),
            pltpu.VMEM((D // 2, NC * XC, 128), u32),
            pltpu.SMEM((1,), f32),
            pltpu.SMEM((2,), jnp.int32),
            pltpu.VMEM((2, 24, TQ), f32),
            pltpu.VMEM((S, TQ), f32),
            pltpu.VMEM((8, TQ), f32),
        ],
        compiler_params=pltpu.CompilerParams(
            dimension_semantics=("arbitrary",),
            vmem_limit_bytes=120 * 1024 * 1024,
        ),
    )(A_x.reshape(S, D), A_wqkv, A_wo, B_w1, B_b1, B_w2, B_b2)
    return out.reshape(1, S, D)
```
